```python
import os as _os
_os.environ.setdefault("JAX_PLATFORMS", "cpu")
import jax
import jax.numpy as jnp

def _softmax(x, axis=-1):
    return jax.nn.softmax(x, axis=axis)
def _gelu(x):
    return jax.nn.gelu(x, approximate=True)
def _silu(x):
    return jax.nn.silu(x)
def _sigmoid(x):
    return jax.nn.sigmoid(x)
def _layernorm(x, axis=-1, eps=1e-5):
    m = jnp.mean(x, axis=axis, keepdims=True)
    v = jnp.var(x, axis=axis, keepdims=True)
    return (x - m) / jnp.sqrt(v + eps)
def _scatter_add(tgt, idx, src, axis=0):
    return tgt.at[idx].add(src)
def _segment_sum(src, seg, n):
    return jax.ops.segment_sum(src, seg, n)
class _Rng:
    def __init__(self, key):
        self._k = key
    def _next(self):
        self._k, sub = jax.random.split(self._k)
        return sub
    def normal(self, shape):
        return jax.random.normal(self._next(), shape, dtype=jnp.bfloat16)
    def randint(self, lo, hi, shape):
        return jax.random.randint(self._next(), shape, lo, hi, dtype=jnp.int32)
    def uniform(self, shape, lo=0.0, hi=1.0):
        return jax.random.uniform(self._next(), shape, jnp.bfloat16, lo, hi)
    def permutation(self, n):
        return jax.random.permutation(self._next(), n)


kernel_name = 'interleave_layers__sliding_block_cached__mixer_channel_mlp__decode'

def setup_inputs():
    _rng = _Rng(jax.random.key(int.from_bytes(__import__("os").urandom(4), "little")))
    _w = (lambda a: (lambda t: t.astype(jnp.bfloat16) if jnp.issubdtype(t.dtype, jnp.floating) else t)(jnp.asarray(a)))
    def _A_setup():
        B, Sq, D = 8, 1, 640
        Hq, Hkv, Sk, Dh = 32, 32, 4096, 128
        assert Hq % Hkv == 0, (Hq, Hkv)
        return {
            "x": _w((lambda *s: _rng.normal(s) * 0.05)(B, Sq, D)),
            "k_cache": _w((lambda *s: _rng.normal(s) * 1.6)(B, Hkv, Sk, Dh)),
            "v_cache": _w((lambda *s: _rng.normal(s) * 0.8)(B, Hkv, Sk, Dh)),
            "wq": _w((lambda *s: _rng.normal(s) * 1.6)(D, Hq * Dh) * (D ** -0.5)),
            "wo": _w((lambda *s: _rng.normal(s) * 0.8)(Hq * Dh, D) * ((Hq * Dh) ** -0.5)),
        }
    _A_in = _A_setup()

    def _B_setup():
        B, S, D, F = 8, 1, 640, 1728
        return {
            "x": _w((lambda *s: _rng.normal(s) * 0.05)(B, S, D)),
            "w1": _w((lambda *s: _rng.normal(s) * 0.4)(D, F) * (D ** -0.5)),
            "b1": _w((lambda *s: _rng.normal(s) * 0.4)(F)),
            "w2": _w((lambda *s: _rng.normal(s) * 0.4)(F, D) * (F ** -0.5)),
            "b2": _w((lambda *s: _rng.normal(s) * 0.2)(D)),
        }
    _B_in = _B_setup()

    return {
        "A_x": _A_in["x"],
        "A_k_cache": _A_in["k_cache"],
        "A_v_cache": _A_in["v_cache"],
        "A_wq": _A_in["wq"],
        "A_wo": _A_in["wo"],
        "B_x": _B_in["x"],
        "B_w1": _B_in["w1"],
        "B_b1": _B_in["b1"],
        "B_w2": _B_in["w2"],
        "B_b2": _B_in["b2"],
    }

def reference(A_x, A_k_cache, A_v_cache, A_wq, A_wo, B_x, B_w1, B_b1, B_w2, B_b2):
    def _A_ref(x, k_cache, v_cache, wq, wo):
        B, Sq, D = x.shape
        Hq, Dh = 32, 128
        Hkv, Sk = k_cache.shape[1], k_cache.shape[2]
        W = min(4096, max(256, Sk // 4))
        rep = Hq // Hkv
        q = (lambda x, *d: x.transpose(*d))((x @ wq).reshape(B, Sq, Hq, Dh), 0, 2, 1, 3)
        k = jnp.repeat(k_cache[:, :, Sk - W:, :], rep, axis=1)
        v = jnp.repeat(v_cache[:, :, Sk - W:, :], rep, axis=1)
        scores = jnp.einsum("bhqd,bhkd->bhqk", q, k) * (Dh ** -0.5)
        p = _softmax(scores, axis=-1)
        o = jnp.einsum("bhqk,bhkd->bhqd", p, v)
        return (lambda x, *d: x.transpose(*d))(o, 0, 2, 1, 3).reshape(B, Sq, Hq * Dh) @ wo

    def _B_ref(x, w1, b1, w2, b2):
        y = _layernorm(x, axis=-1)
        h = _gelu(jnp.einsum("bsd,df->bsf", y, w1) + b1)
        return jnp.einsum("bsf,fd->bsd", h, w2) + b2

    x = A_x
    x = x + _A_ref(_layernorm(x, axis=-1), A_k_cache, A_v_cache, A_wq, A_wo)
    x = x + _B_ref(_layernorm(x, axis=-1), B_w1, B_b1, B_w2, B_b2)
    x = x + _A_ref(_layernorm(x, axis=-1), A_k_cache, A_v_cache, A_wq, A_wo)
    x = x + _B_ref(_layernorm(x, axis=-1), B_w1, B_b1, B_w2, B_b2)
    return x
```

```python
import functools, math
import jax, jax.numpy as jnp
from jax import lax
from jax.experimental import pallas as pl
from jax.experimental.pallas import tpu as pltpu

B, D, H, DH, SK, W, F = 8, 640, 32, 128, 4096, 1024, 1728
G = 8
NG = H // G
NT = (((1,), (1,)), ((), ()))
NN = (((1,), (0,)), ((), ()))
f32, bf16, i32 = jnp.float32, jnp.bfloat16, jnp.int32
EXP_SCALE = (DH ** -0.5) * math.log2(math.e)

def _ln(x):
    m = jnp.mean(x, axis=-1, keepdims=True)
    c = x - m
    v = jnp.mean(c * c, axis=-1, keepdims=True)
    return c * lax.rsqrt(v + 1e-5)

def _gelu(x):
    return 0.5 * x * (1.0 + jnp.tanh(math.sqrt(2.0 / math.pi) * (x + 0.044715 * (x * x * x))))

def make(bounds=False, lead=2, wmode="simple"):
    def kern(x_hbm, k_hbm, v_hbm, wq_hbm, wo_hbm, w1_hbm, b1_hbm, w2_hbm, b2_hbm, o_ref,
             kv, wq, wo, w1, w2, xv, b1v, b2v, xs, q3, acc, sems, wsems):
        k32 = k_hbm.bitcast(i32)
        v32 = v_hbm.bitcast(i32)
        row = lax.broadcasted_iota(i32, (G, DH), 0)
        rowd = lax.broadcasted_iota(i32, (B, D), 0)

        def unit_pieces(b, g, t):
            slot = b % 2
            src = (k32, v32)[t]
            out = []
            for n in range(64):
                r, hh = n // 2, n % 2
                def go(r=r, hh=hh):
                    pltpu.make_async_copy(
                        src.at[b, pl.ds(g * G + hh * 4, 4), pl.ds((SK - W) // 2 + r * 16, 16)],
                        kv.at[slot, t, pl.ds(g * G + hh * 4, 4), pl.ds(r * 16, 16)],
                        sems.at[slot, t, g]).start(priority=hh)
                out.append(go)
            return out

        def unit_wait(b, g, t):
            slot = b % 2
            ref = kv.at[slot, t, pl.ds(g * G, G)]
            pltpu.make_async_copy(ref, ref, sems.at[slot, t, g]).wait()

        def ld(ref, *idx):
            return pltpu.bitcast(ref[idx], bf16)

        small = [pltpu.make_async_copy(x_hbm, xv, wsems.at[0]),
                 pltpu.make_async_copy(b1_hbm, b1v, wsems.at[1]),
                 pltpu.make_async_copy(b2_hbm, b2v, wsems.at[2])]
        big = [pltpu.make_async_copy(wq_hbm.bitcast(i32), wq, wsems.at[3]),
               pltpu.make_async_copy(wo_hbm.bitcast(i32), wo, wsems.at[4]),
               pltpu.make_async_copy(w1_hbm.bitcast(i32), w1, wsems.at[5]),
               pltpu.make_async_copy(w2_hbm.bitcast(i32), w2, wsems.at[6])]
        for c in small: c.start()
        for c in big: c.start()

        def project_q():
            y = _ln(xs[...]).astype(bf16)
            for c in range(4):
                q = lax.dot_general(y, pltpu.bitcast(wq[:, c * 1024:(c + 1) * 1024], bf16), NN, preferred_element_type=f32)
                for j in range(8):
                    q3[:, c * 8 + j, :] = q[:, j * 128:(j + 1) * 128]

        def attend(b, g, a, issue=()):
            slot = b % 2
            issue = list(issue)
            per = len(issue) // (2 * G)
            def tick():
                for _ in range(per): issue.pop(0)()
            h0 = pl.multiple_of(g * G, G)
            qg = q3[b, pl.ds(h0, G), :].astype(bf16)
            s = [None] * 8
            for h in range(G):
                sh = lax.dot_general(qg, ld(kv, slot, 0, h0 + h), NT, preferred_element_type=f32)
                for j in range(8):
                    t = sh[:, j * 128:(j + 1) * 128]
                    s[j] = t if h == 0 else jnp.where(row == h, t, s[j])
                tick()
            s = jnp.concatenate(s, axis=1)
            m = jnp.max(s, axis=1, keepdims=True)
            p = jnp.exp2((s - m) * EXP_SCALE)
            l = jnp.sum(p, axis=1, keepdims=True)
            pb = p.astype(bf16)
            o = None
            for h in range(G):
                t = lax.dot_general(pb, ld(kv, slot, 1, h0 + h), NN, preferred_element_type=f32)
                o = t if h == 0 else jnp.where(row == h, t, o)
                tick()
            ob = (o / l).astype(bf16)
            r = None
            for h in range(G):
                wo_h = pltpu.bitcast(wo[pl.ds(pl.multiple_of((h0 + h) * 64, 64), 64), :], bf16)
                t = lax.dot_general(ob, wo_h, NN, preferred_element_type=f32)
                r = t if h == 0 else jnp.where(rowd == h, t, r)
            acc[a] += r
            assert not issue

        def transition(s):
            a1 = jnp.sum(acc[0], axis=0, keepdims=True)
            a2 = jnp.sum(acc[1], axis=0, keepdims=True)
            acc[...] = jnp.zeros_like(acc)
            x0 = xs[...]
            x1 = x0 + jnp.where(rowd == s, a1, a2)
            y = _ln(_ln(x1)).astype(bf16)
            hid = lax.dot_general(y, pltpu.bitcast(w1[...], bf16), NT, preferred_element_type=f32)
            hid = _gelu(hid + b1v[...].astype(f32).reshape(1, F)).astype(bf16)
            z = lax.dot_general(hid, pltpu.bitcast(w2[...], bf16), NN, preferred_element_type=f32)
            x2 = x1 + z + b2v[...].astype(f32).reshape(1, D)
            xs[...] = jnp.where((rowd == s) | (rowd == s - 1), x2, x0)

        for u in range(4 + lead):
            for go in unit_pieces(u // 8, (u // 2) % 4, u % 2): go()
        acc[...] = jnp.zeros_like(acc)
        for c in small: c.wait()
        xs[...] = xv[...].astype(f32)
        big[0].wait()
        project_q()
        for c in big[1:]: c.wait()

        def body(jj, _):
            for t in range(2):
                j = jj * 2 + t
                s, i = j // 8, j % 8
                l1 = i >= 4
                b = jnp.where(l1, s, s - 1)
                g = i % 4
                @pl.when(l1)
                def _():
                    unit_wait(b, g, 0)
                    unit_wait(b, g, 1)
                u = j + lead
                attend(b, g, jnp.where(l1, 0, 1), unit_pieces(u // 8, (u // 2) % 4, (t + lead) % 2))
            @pl.when(jj % 4 == 3)
            def _():
                transition(jj // 4)
                project_q()
        assert lead % 2 == 0
        lax.fori_loop(2, (64 - lead) // 2, body, None)

        for j in range(64 - lead, 64):
            g = j % 4
            unit_wait(7, g, 0)
            unit_wait(7, g, 1)
            attend(7, g, 0)
        transition(7)
        project_q()
        def l2(g, _):
            attend(7, g, 1)
        lax.fori_loop(0, 4, l2, None)
        transition(8)
        o_ref[...] = xs[...].astype(bf16)

    def fn(A_x, K, V, A_wq, A_wo, B_x, B_w1, B_b1, B_w2, B_b2):
        out = pl.pallas_call(
            kern,
            in_specs=[pl.BlockSpec(memory_space=pl.ANY)] * 9,
            out_specs=pl.BlockSpec(memory_space=pltpu.VMEM),
            out_shape=jax.ShapeDtypeStruct((B, D), bf16),
            scratch_shapes=[
                pltpu.VMEM((2, 2, H, W // 2, DH), i32),
                pltpu.VMEM((D // 2, H * DH), i32), pltpu.VMEM((H * DH // 2, D), i32),
                pltpu.VMEM((F // 2, D), i32), pltpu.VMEM((F // 2, D), i32),
                pltpu.VMEM((B, D), bf16), pltpu.VMEM((F,), bf16), pltpu.VMEM((D,), bf16),
                pltpu.VMEM((B, D), f32), pltpu.VMEM((B, H, DH), f32), pltpu.VMEM((2, G, D), f32),
                pltpu.SemaphoreType.DMA((2, 2, NG)), pltpu.SemaphoreType.DMA((7,)),
            ],
            compiler_params=pltpu.CompilerParams(vmem_limit_bytes=100 * 1024 * 1024,
                                                 disable_bounds_checks=not bounds),
        )(A_x.reshape(B, D), K, V, A_wq, A_wo, B_w1.T, B_b1, B_w2, B_b2)
        return out.reshape(B, 1, D)
    return fn


@jax.jit
def pallas_interleave_layers__sliding_block_cached__mixer_channel_mlp__decode_kernel(
    A_x, A_k_cache, A_v_cache, A_wq, A_wo, B_x, B_w1, B_b1, B_w2, B_b2,
):
    return make(lead=4)(A_x, A_k_cache, A_v_cache, A_wq, A_wo, B_x, B_w1, B_b1, B_w2, B_b2)
```

```python
import functools
import math

import jax
import jax.numpy as jnp
from jax import lax
import jax.experimental.pallas as pl
import jax.experimental.pallas.tpu as pltpu

f32, bf16, i32 = jnp.float32, jnp.bfloat16, jnp.int32

B, D, H, DH, SK, F = 8, 640, 32, 128, 4096, 1728
W = min(4096, max(256, SK // 4))
FP = 1792
G = 8
EPS = 1e-5
EXP2_SCALE = DH ** -0.5 * math.log2(math.e)
GELU_C = math.sqrt(2.0 / math.pi)

PAIRS_ATTN = 20
PAIRS_MLP = 24
PAIRS_REST = 256 - 8 * PAIRS_ATTN - PAIRS_MLP
LEAD = 128 - PAIRS_ATTN - PAIRS_MLP
LAST_HEADS = ((16, 4), (20, 4), (24, 5), (29, 2), (31, 1))

UP_MXU = 6
DOWN_MXU = 11
Q_MXU = (0, 1, 2)
O_MXU = (29, 30, 31)
PV_VPU = (0, 1, 2, 4, 6, 10, 11, 12, 14)
SOFTMAX_GROUPS = (4, 4, 8, 8, 8)
KT_PAD, WQ_PAD = 128, 384

SCRATCH = dict(
    k=((2 * H, W // 2, DH), i32),
    v=((2 * H, W // 2, DH), i32),
    kt_a=((H - G, DH // 2, W + KT_PAD), i32),
    kt_b=((G, DH // 2, W + KT_PAD), i32),
    wq_in=((4, D // 4, H * DH), bf16),
    wo_in=((4, H * DH // 4, D), bf16),
    w1_in=((3, F // 3, D), bf16),
    w2_in=((3, F // 3, D), bf16),
    wq=((D // 2, H * DH + WQ_PAD), i32),
    wo=((H * DH // 2, D), i32),
    w1=((D // 2, FP), i32),
    w2=((FP // 2, D), i32),
    wq_t_f32=((H * DH, D), f32),
    wo_f32=((H * DH, D), f32),
    w1_t_f32=((F - 128 * UP_MXU, D), f32),
    w1_sum=((B, FP), f32),
    wq_sum=((B, H * DH), f32),
    w2_half_f32=((F - 128 * DOWN_MXU, D), f32),
    b1_col=((FP - 128 * DOWN_MXU, 128), f32),
    x_in=((B, D), bf16),
    b1_in=((F,), bf16),
    b2_in=((D,), bf16),
    b1=((B, FP), f32),
    b2=((B, D), f32),
    x=((B, D), f32),
    out=((B, D), bf16),
    w1_sum_col=((FP - 128 * DOWN_MXU, 128), f32),
    q=((H * B + B, DH), f32),
    acc=((2, G, D), f32),
    vt_f32=((len(PV_VPU), DH, W), f32),
)


def _dot(a, b, transpose_b=False):
    dims = (((1,), (1 if transpose_b else 0,)), ((), ()))
    return lax.dot_general(a, b, dims, preferred_element_type=f32)


def _bf16(words):
    return pltpu.bitcast(words, bf16)


def _words(x):
    return pltpu.bitcast(x, i32)


def _tiles(x):
    return [x[:, k * 128:(k + 1) * 128] for k in range(x.shape[1] // 128)]


def _tile(ref, k):
    return ref[:, k * 128:(k + 1) * 128]


def _chain_sum(xs):
    return functools.reduce(lambda a, b: a + b, xs)


def _tree_sum(xs):
    while len(xs) > 1:
        xs = [_chain_sum(xs[i:i + 2]) for i in range(0, len(xs), 2)]
    return xs[0]


def _row_sum(x):
    return jnp.broadcast_to(jnp.sum(x, axis=0, keepdims=True), x.shape)


def _lane_sum(x):
    return jnp.broadcast_to(jnp.sum(x, axis=1, keepdims=True), x.shape)


def _row(x, j):
    return jnp.broadcast_to(x[j:j + 1, :], x.shape)


def _layernorm(x):
    c = x - jnp.mean(x, axis=-1, keepdims=True)
    return c * lax.rsqrt(jnp.mean(c * c, axis=-1, keepdims=True) + EPS)


def _gelu_twice(x):
    return x * jnp.tanh(x * (x * x * (GELU_C * 0.044715) + GELU_C)) + x


def _mean_var(x):
    xt = _tiles(x)
    mean = _lane_sum(_tree_sum(xt)) * (1.0 / D)
    return mean, _lane_sum(_tree_sum([(t - mean) * (t - mean) for t in xt])) * (1.0 / D)


def _emit_interleaved(tasks):
    users = {t[1]: [] for t in tasks}
    for t in tasks:
        for dep, latency in t[4]:
            users[dep].append((t[1], latency))
    clock, done, todo, plan = {"M": 0, "V": 0}, {}, list(tasks), []
    while todo:
        best = None
        for t in todo:
            if all(u in done for u, _ in users[t[1]]):
                key = (max([clock[t[0]]] + [done[u] + lat for u, lat in users[t[1]]]), -t[3])
                if best is None or key < best[0]:
                    best = (key, t)
        (time, _), t = best
        todo.remove(t)
        clock[t[0]] = done[t[1]] = time + t[2]
        plan.append((time + t[2], len(plan), t))
    for _, _, t in sorted(plan, key=lambda e: e[:2], reverse=True):
        t[5]()


def _mlp_one_row(x, r):
    mean, var = _mean_var(x)
    xt = _tiles(x)
    s1 = lax.rsqrt(var + EPS)
    scale = s1 * lax.rsqrt(var * s1 * s1 + EPS)
    xb = x.astype(bf16)
    hid, part, pre, z_m, z_v = {}, {}, {}, {}, {}

    def activate(j, t):
        hid[j] = 0.5 * _gelu_twice((t - mean * _tile(r["w1_sum"], j)) * scale + _tile(r["b1"], j))

    def up_rows(u):
        return _chain_sum([r["w1_t_f32"][u * 8:(u + 1) * 8, k * 128:(k + 1) * 128] * xt[k] for k in range(5)])

    def up_m(j):
        activate(j, _dot(xb, _bf16(_tile(r["w1"], j))))

    def up_v(j):
        part[j] = jnp.concatenate([up_rows((j - UP_MXU) * 16 + u) for u in range(16)], axis=0).T

    def up_v_finish(j):
        activate(j, _row_sum(_chain_sum([part[j][u * 8:(u + 1) * 8] for u in range(16)])))

    def down_m(j):
        for k, t in enumerate(_tiles(_dot(hid[j].astype(bf16), _bf16(r["w2"][j * 64:(j + 1) * 64, :])))):
            z_m[k] = t if k not in z_m else z_m[k] + t

    def up_col(us):
        for u in us:
            pre[u] = _lane_sum(up_rows((DOWN_MXU - UP_MXU) * 16 + u))

    def down_v(us):
        for u in us:
            rows = slice(u * 8, (u + 1) * 8)
            h = _gelu_twice((pre[u] - mean * r["w1_sum_col"][rows, :]) * scale + r["b1_col"][rows, :])
            for k in range(5):
                t = r["w2_half_f32"][rows, k * 128:(k + 1) * 128] * h
                z_v[k, u % 2] = t if (k, u % 2) not in z_v else z_v[k, u % 2] + t

    bind, tasks = functools.partial, []
    for j in range(UP_MXU):
        tasks.append(("M", f"a{j}", 40, j, [], bind(up_m, j)))
        tasks.append(("M", f"b{j}", 40, 100 + j, [(f"a{j}", 70)], bind(down_m, j)))
    for j in range(UP_MXU, DOWN_MXU):
        tasks.append(("V", f"t{j}", 37, j, [], bind(up_v, j)))
        tasks.append(("V", f"a{j}", 8, j - 50, [(f"t{j}", 90)], bind(up_v_finish, j)))
        tasks.append(("M", f"b{j}", 40, 100 + j, [(f"a{j}", 70)], bind(down_m, j)))
    n = (F - DOWN_MXU * 128) // 16
    for i in range(n + 1):
        if i < n:
            tasks.append(("V", f"c{i}", 5, DOWN_MXU - 4 + i / 8, [], bind(up_col, (2 * i, 2 * i + 1))))
        if i > 0:
            tasks.append(("V", f"d{i}", 10, DOWN_MXU - 4 + (i + 0.5) / 8, [(f"c{i - 1}", 0)],
                          bind(down_v, (2 * i - 2, 2 * i - 1))))
    _emit_interleaved(tasks)
    base = _tiles(x + r["b2"][...])
    return jnp.concatenate([base[k] + _row_sum(z_v[k, 0] + z_v[k, 1]) + z_m[k] for k in range(5)], axis=1)


def _keys_t(r, h):
    return _bf16(r["kt_a"][h, :, :W] if h < H - G else r["kt_b"][h - (H - G), :, :W])


def _attention_one_row(x, r):
    row = lax.broadcasted_iota(i32, (8, 128), 0)
    mean, var = _mean_var(x)
    scale = lax.rsqrt(var + EPS) * EXP2_SCALE
    xb, xt = x.astype(bf16), _tiles(x)
    q, part, s, p, o, col, p_rows, z = {}, {}, {}, {}, {}, {}, {}, {}
    groups, place = [], {}
    for g, n in enumerate(SOFTMAX_GROUPS):
        groups.append(list(range(len(place), len(place) + n)))
        place.update({h: (g, j) for j, h in enumerate(groups[-1])})

    def diagonal(ts):
        out = ts[0]
        for k in range(1, len(ts)):
            out = jnp.where(row == k, ts[k], out)
        return out

    def add(key, t):
        z[key] = t if key not in z else z[key] + t

    def query_m(h):
        q[h] = _dot(xb, _bf16(_tile(r["wq"], h))) - mean * _tile(r["wq_sum"], h)

    def query_v(h):
        def rows(u):
            n = h * DH + u * 8
            return _chain_sum([r["wq_t_f32"][n:n + 8, k * 128:(k + 1) * 128] * xt[k] for k in range(5)])
        part[h] = jnp.concatenate([rows(u) for u in range(16)], axis=0).T

    def query_v_finish(h):
        t = _row_sum(_chain_sum([part[h][u * 8:(u + 1) * 8] for u in range(16)]))
        q[h] = t - mean * _tile(r["wq_sum"], h)

    def scores(h):
        s[h] = diagonal(_tiles(_dot(q[h].astype(bf16), _keys_t(r, h))))

    def softmax(hs):
        m = diagonal([jnp.broadcast_to(jnp.max(s[h], axis=0, keepdims=True), (8, 128)) for h in hs])
        m = jnp.broadcast_to(jnp.max(m, axis=1, keepdims=True), (8, 128))
        e = [jnp.exp2((s[h] - m[j:j + 1, :]) * scale) for j, h in enumerate(hs)]
        inv = 1.0 / _lane_sum(diagonal([_row_sum(t) for t in e]))
        for j, h in enumerate(hs):
            p[h] = (e[j], inv)

    def values_m(h):
        j = place[h][1]
        pb = p[h][0].astype(bf16)
        t = diagonal([_dot(pb, _bf16(r["v"][H + h, k * 64:(k + 1) * 64, :])) for k in range(8)])
        t = t * p[h][1][j:j + 1, :]
        o[h] = t if h in O_MXU else _row_sum(t)

    def values_v(h, i):
        if i == 0:
            j = place[h][1]
            e = p[h][0] * p[h][1][j:j + 1, :]
            p_rows[h] = [_row(e, k) for k in range(8)]
        for u in range(4 * i, 4 * i + 4):
            t = [r["vt_f32"][PV_VPU.index(h), u * 8:(u + 1) * 8, k * 128:(k + 1) * 128] * p_rows[h][k]
                 for k in range(8)]
            col[h, u] = _lane_sum(_chain_sum(t[:4]) + _chain_sum(t[4:]))

    def to_columns(h):
        t = jnp.concatenate([o[h]] * 16, axis=0).T
        for u in range(16):
            col[h, u] = t[u * 8:(u + 1) * 8]

    def output_m(h):
        for k, t in enumerate(_tiles(_dot(o[h].astype(bf16), _bf16(r["wo"][h * 64:(h + 1) * 64, :])))):
            add((k, "M"), t)

    def output_v(h, us):
        for u in us:
            n = h * DH + u * 8
            for k in range(5):
                add((k, "V"), r["wo_f32"][n:n + 8, k * 128:(k + 1) * 128] * col[h, u])

    bind, tasks = functools.partial, []
    for h in range(H):
        ready = [(f"p{place[h][0]}", 145)]
        if h in Q_MXU:
            tasks.append(("M", f"q{h}", 40, h - 3, [], bind(query_m, h)))
        else:
            tasks.append(("V", f"Q{h}", 40, h - 1, [], bind(query_v, h)))
            tasks.append(("V", f"q{h}", 6, h - 2, [(f"Q{h}", 160)], bind(query_v_finish, h)))
        tasks.append(("M", f"s{h}", 64, h, [(f"q{h}", 100 if h in Q_MXU else 10)], bind(scores, h)))
        if h in PV_VPU:
            for i in range(4):
                tasks.append(("V", f"w{h}_{i}", 15.5, h + 5 + i / 10, [(f"w{h}_{i - 1}", 0)] if i else ready,
                              bind(values_v, h, i)))
                tasks.append(("V", f"x{h}_{i}", 10, h - 45,
                              [(f"w{h}_{i}", 80)] + ([(f"x{h}_{i - 1}", 0)] if i else []),
                              bind(output_v, h, range(4 * i, 4 * i + 4))))
            continue
        tasks.append(("M", f"v{h}", 64, h + 40, ready, bind(values_m, h)))
        if h in O_MXU:
            tasks.append(("M", f"o{h}", 40, h + 100, [(f"v{h}", 130)], bind(output_m, h)))
        else:
            tasks.append(("V", f"c{h}", 2, h + 4, [(f"v{h}", 130)], bind(to_columns, h)))
            tasks.append(("V", f"o{h}", 40, h + 10, [(f"c{h}", 160)], bind(output_v, h, range(16))))
    for g, hs in enumerate(groups):
        tasks.append(("V", f"p{g}", 12, 1000, [(f"s{h}", 90) for h in hs], bind(softmax, hs)))
    _emit_interleaved(tasks)
    return x + jnp.concatenate([_row_sum(z[k, "V"] + z[k, "M"]) for k in range(5)], axis=1)


def _kernel(x_hbm, k_hbm, v_hbm, wq_hbm, wo_hbm, w1_hbm, b1_hbm, w2_hbm, b2_hbm, out_hbm, *scratch):
    r = dict(zip(SCRATCH, scratch))
    kv_sems, w_sems, last_sems, fence_sem = scratch[len(SCRATCH):]
    copy = pltpu.make_async_copy
    window = (SK - W) // 2
    kv_src = (k_hbm.bitcast(i32), v_hbm.bitcast(i32))
    kv_dst = (r["k"], r["v"])
    row = lax.broadcasted_iota(i32, (G, DH), 0)
    row_d = lax.broadcasted_iota(i32, (B, D), 0)

    def start_pair(m):
        group, h, w = m >> 6, (m & 3) * 2, ((m >> 2) & 15) * 32
        if not isinstance(w, int):
            w = pl.multiple_of(w, 32)
        for t in range(2):
            copy(kv_src[t].at[pl.ds(group * G + h, 2), pl.ds(window + w, 32)],
                 kv_dst[t].at[pl.ds((group & 7) * G + h, 2), pl.ds(w, 32)],
                 kv_sems.at[t, group & 7]).start(priority=t)

    def start_pairs(m, n):
        def body(i, _):
            for c in range(4):
                start_pair(m + i * 4 + c)
        lax.fori_loop(0, n // 4, body, None)

    def spread_pairs(m, n, points):
        calls = [0]
        def tick():
            for c in range(n * calls[0] // points, n * (calls[0] + 1) // points):
                start_pair(m + c)
            calls[0] += 1
        return tick

    def wait_group(t, group):
        ref = kv_dst[t].at[pl.ds((group & 7) * G, G)]
        copy(ref, ref, kv_sems.at[t, group & 7]).wait()

    def idle():
        pass

    def queries(b, g):
        return r["q"][pl.ds(g * (G * B) + b, G, stride=B), :].astype(bf16)

    def probabilities(q, keys, transpose, tick):
        s = [None] * (W // 128)
        for h in range(G):
            for j, t in enumerate(_tiles(_dot(q, keys(h), transpose))):
                s[j] = t if h == 0 else jnp.where(row == h, t, s[j])
            tick()
        s = jnp.concatenate(s, axis=1)
        p = jnp.exp2((s - jnp.max(s, axis=1, keepdims=True)) * EXP2_SCALE)
        return p.astype(bf16), jnp.sum(p, axis=1, keepdims=True)

    def outputs(p, slot, g, heads, tick):
        o = None
        for h in heads:
            t = _dot(p[0], _bf16(r["v"][slot + h]))
            o = t if o is None else jnp.where(row == h, t, o)
            tick()
        o = (o / p[1]).astype(bf16)
        out = None if len(heads) == G else jnp.zeros((G, D), f32)
        for h in heads:
            w = (g * G + h) * 64
            if not isinstance(w, int):
                w = pl.multiple_of(w, 64)
            t = _dot(o, _bf16(r["wo"][pl.ds(w, 64), :]))
            out = t if out is None else jnp.where(row_d == h, t, out)
            tick()
        return out

    def mlp(x, tick):
        y = _layernorm(_layernorm(x)).astype(bf16)
        edges = [(c, min(c + 512, FP)) for c in range(0, FP, 512)]
        hid = []
        for lo, hi in edges:
            hid.append((0.5 * _gelu_twice(_dot(y, _bf16(r["w1"][:, lo:hi])) + r["b1"][:, lo:hi])).astype(bf16))
            tick()
        out = x + r["b2"][...]
        for h, (lo, hi) in zip(hid, edges):
            out = out + _dot(h, _bf16(r["w2"][lo // 2:hi // 2, :]))
            tick()
        return out

    def project_queries(tick):
        y = _layernorm(r["x"][...]).astype(bf16)
        for c in range(8):
            for j, t in enumerate(_tiles(_dot(y, _bf16(r["wq"][:, c * 512:(c + 1) * 512])))):
                r["q"][(c * 4 + j) * B:(c * 4 + j + 1) * B, :] = t
            tick()

    def load_wq_wo(i, _):
        rows = pl.ds(pl.multiple_of((i >> 3) * 8, 8), 8)
        cols = pl.ds(pl.multiple_of((i & 7) * 512, 512), 512)
        copy(wq_hbm.at[:, rows, cols], r["wq_in"].at[:, rows, cols], w_sems.at[3]).start(priority=0)

        @pl.when(i < H * DH // 4 // 8)
        def _():
            rows = pl.ds(pl.multiple_of(i * 8, 8), 8)
            copy(wo_hbm.at[:, rows], r["wo_in"].at[:, rows], w_sems.at[4]).start(priority=1)

    def load_w1_w2(i, _):
        rows = pl.ds(pl.multiple_of(i * 8, 8), 8)
        copy(w1_hbm.at[:, rows], r["w1_in"].at[:, rows], w_sems.at[5]).start(priority=0)
        copy(w2_hbm.at[:, rows], r["w2_in"].at[:, rows], w_sems.at[6]).start(priority=1)

    small = [copy(x_hbm, r["x_in"], w_sems.at[0]), copy(b1_hbm, r["b1_in"], w_sems.at[1]),
             copy(b2_hbm, r["b2_in"], w_sems.at[2])]
    lax.fori_loop(0, D // 4, load_wq_wo, None)
    for c in small:
        c.start()
    lax.fori_loop(0, F // 3 // 8, load_w1_w2, None)

    def wait_weight(name, i):
        copy(r[name], r[name], w_sems.at[i]).wait()

    def columns(ref, bias):
        for j in range(DOWN_MXU, FP // 128):
            t = jnp.broadcast_to(bias[0:1, j * 128:(j + 1) * 128], (128, 128)).T
            ref[(j - DOWN_MXU) * 128:(j - DOWN_MXU + 1) * 128, :] = t

    for c in small:
        c.wait()
    r["acc"][...] = jnp.zeros((2, G, D), f32)
    r["q"][H * B:, :] = jnp.zeros((B, DH), f32)
    r["x"][...] = r["x_in"][...].astype(f32)
    b1 = jnp.concatenate([r["b1_in"][...].astype(f32).reshape(1, F), jnp.zeros((1, FP - F), f32)], axis=1)
    r["b1"][...] = jnp.broadcast_to(b1, (B, FP))
    columns(r["b1_col"], b1)
    r["b2"][...] = jnp.broadcast_to(r["b2_in"][...].astype(f32).reshape(1, D), (B, D))

    def pack_wq(i, _):
        for a in range(4):
            rows = pl.ds(pl.multiple_of(a * (D // 8) + i * 8, 8), 8)
            r["wq"][rows, :H * DH] = _words(r["wq_in"][a, pl.ds(pl.multiple_of(i * 16, 16), 16), :])
            if a % 2:
                start_pair(i * 2 + a // 2)

    def transpose_wq(i, _):
        for e in range(2):
            head = pl.ds(pl.multiple_of((2 * i + e) * DH, DH), DH)
            r["wq_t_f32"][head, :] = _bf16(r["wq"][:, head]).T.astype(f32)
            for c in range(2 + 2 * e):
                start_pair(36 + i * 6 + 2 * e + c)

    def pack_wo(i, _):
        for a in range(4):
            w = r["wo_in"][a, pl.ds(pl.multiple_of(i * DH, DH), DH), :]
            r["wo"][pl.ds(pl.multiple_of((a * 8 + i) * 64, 64), 64), :] = _words(w)
            r["wo_f32"][pl.ds(pl.multiple_of((a * 8 + i) * DH, DH), DH), :] = w.astype(f32)
            start_pair(132 + i * 4 + a)

    wait_weight("wq_in", 3)
    lax.fori_loop(0, 10, pack_wq, None)
    project_queries(spread_pairs(20, 16, 8))
    lax.fori_loop(0, H // 2, transpose_wq, None)
    wait_weight("wo_in", 4)
    lax.fori_loop(0, 8, pack_wo, None)

    def mlp_rows(name, n):
        return r[name][n // (F // 3), n % (F // 3):n % (F // 3) + 64, :]

    loop_start = LEAD + 256 - PAIRS_REST - 3 * PAIRS_ATTN
    tick = spread_pairs(164, loop_start - 164, 9 + 14 + 8)
    wait_weight("w2_in", 6)
    for n in range(0, F, 64):
        w = mlp_rows("w2_in", n)
        r["w2"][n // 2:n // 2 + 32, :] = _words(w)
        if n >= 128 * DOWN_MXU:
            r["w2_half_f32"][n - 128 * DOWN_MXU:n - 128 * DOWN_MXU + 64, :] = 0.5 * w.astype(f32)
        if n % 192 == 0:
            tick()
    r["w2"][F // 2:, :] = jnp.zeros(((FP - F) // 2, D), i32)
    wait_weight("w1_in", 5)
    for c in range(FP // 128):
        halves = []
        for n in (c * 128, c * 128 + 64):
            halves.append(mlp_rows("w1_in", n) if n < F else jnp.zeros((64, D), bf16))
            if 128 * UP_MXU <= n < F:
                r["w1_t_f32"][n - 128 * UP_MXU:n - 128 * UP_MXU + 64, :] = halves[-1].astype(f32)
        r["w1"][:, c * 128:(c + 1) * 128] = _words(jnp.concatenate(halves, axis=0).T)
        tick()
    ones = jnp.ones((B, D), bf16)
    w1_sum = _dot(ones, _bf16(r["w1"][...]))
    r["w1_sum"][...] = w1_sum
    columns(r["w1_sum_col"], w1_sum)
    for c in range(8):
        r["wq_sum"][:, c * 512:(c + 1) * 512] = _dot(ones, _bf16(r["wq"][:, c * 512:(c + 1) * 512]))
        tick()

    def step(j, total):
        s, i = j >> 3, j & 7
        first = i >= 4
        b, g = jnp.where(first, s, s - 1), i & 3
        m = LEAD + 256 * (s + 1) + PAIRS_ATTN * (i - 7)

        @pl.when(i == 7)
        def _():
            start_pairs(m - PAIRS_REST, PAIRS_REST)

        @pl.when(first)
        def _():
            wait_group(0, b * 4 + g)
            wait_group(1, b * 4 + g)

        tick = spread_pairs(jnp.where(i == 7, m, m - PAIRS_REST), PAIRS_ATTN, 3 * G)
        slot = (b & 1) * H + g * G
        p = probabilities(queries(b, g), lambda h: _bf16(r["k"][slot + h]), True, tick)
        r["acc"][jnp.where(first, 0, 1)] += outputs(p, slot, g, range(G), tick)

        @pl.when(i == 7)
        def _():
            tick = spread_pairs(m + PAIRS_ATTN, PAIRS_MLP, 16)
            a1 = jnp.sum(r["acc"][0], axis=0, keepdims=True)
            a2 = jnp.sum(r["acc"][1], axis=0, keepdims=True)
            x = r["x"][...]
            r["acc"][...] = jnp.zeros((2, G, D), f32)
            y = mlp(x + jnp.where(row_d == s, a1, a2), tick)
            r["x"][...] = jnp.where((row_d == s) | (row_d == s - 1), y, x)
            project_queries(tick)

        return total + j

    zero = lax.fori_loop(4, 8 * (B - 1), step, 0) - sum(range(4, 8 * (B - 1)))

    queue = []

    def plan(t, h, n, w, rows, sem, thread):
        c = copy(kv_src[t].at[pl.ds((B - 1) * H + h, n), pl.ds(window + w, rows)],
                 kv_dst[t].at[pl.ds(H + h, n), pl.ds(w, rows)], sem)
        queue.append(functools.partial(c.start, priority=thread))

    def values_sem(h):
        return last_sems.at[2 + [h0 <= h < h0 + n for h0, n in LAST_HEADS].index(True)]

    def wait_heads(t, h, n, sem):
        ref = kv_dst[t].at[pl.ds(H + h, n)]
        copy(ref, ref, sem).wait()

    for e in range(2):
        for i in range(32):
            for thread in range(2):
                plan(0, 16 + 8 * e + 4 * thread + 2 * (i % 2), 2, 32 * (i // 2), 32, last_sems.at[e], thread)
    for i in range(32):
        for thread in range(2):
            plan(1, 16 + 4 * thread + 2 * (i % 2), 2, 32 * (i // 2), 32, values_sem(16 + 4 * thread), thread)
    for i in range(32):
        plan(1, 24 + 2 * (i % 2), 2, 32 * (i // 2), 32, values_sem(24), 0)
        plan(1, 28 + i // 8, 1, 64 * (i % 8), 64, values_sem(28 + i // 8), 1)

    def transpose_keys(h):
        ref = r["kt_a"] if h < H - G else r["kt_b"]
        ref[zero + h % (H - G), :, :W] = _words(_bf16(r["k"][H + h]).T)

    def transpose_values(h):
        r["vt_f32"][zero + PV_VPU.index(h)] = _bf16(r["v"][H + h]).T.astype(f32)

    def spread_queue(pairs, points, side_job=None, heads=(), every=1):
        calls, heads = [0], list(heads)
        def tick():
            for _ in range(2 * (pairs * (calls[0] + 1) // points - pairs * calls[0] // points)):
                queue.pop(0)()
            if heads and calls[0] % every == 0:
                side_job(heads.pop(0))
            calls[0] += 1
        return tick

    def p_prev(g, tick):
        return probabilities(queries(B - 2, g), lambda h: _bf16(r["k"][g * G + h]), True, tick)

    p0 = p_prev(0, spread_queue(9, G))
    wait_group(0, 4 * (B - 1))
    tick = spread_queue(27, 4 * G, transpose_keys, range(G), 4)
    p1 = p_prev(1, tick)
    a = outputs(p0, 0, 0, range(G), tick)
    p2 = p_prev(2, tick)
    wait_group(0, 4 * (B - 1) + 1)
    tick = spread_queue(32, 7 * G, transpose_keys, range(G, 2 * G), 7)
    a = a + outputs(p1, G, 1, range(G), tick)
    p3 = p_prev(3, tick)
    a = a + outputs(p2, 2 * G, 2, range(G), tick) + outputs(p3, 3 * G, 3, range(G), tick)

    def p_last(g, tick):
        return probabilities(queries(B - 1, g), lambda h: _keys_t(r, g * G + h), False, tick)

    wait_group(1, 4 * (B - 1))
    wait_group(1, 4 * (B - 1) + 1)
    tick = spread_queue(18, 2 * G, transpose_values, PV_VPU)
    p0, p1 = p_last(0, tick), p_last(1, tick)
    x = r["x"][...]
    r["x"][...] = jnp.where(row_d == B - 2, mlp(x + jnp.sum(a, axis=0, keepdims=True), idle), x)
    wait_heads(0, 16, G, last_sems.at[0])
    tick = spread_queue(18, 4 * G, transpose_keys, range(2 * G, 3 * G), 4)
    a = outputs(p0, H, 0, range(G), tick) + outputs(p1, H + G, 1, range(G), tick)
    while queue:
        queue.pop(0)()
    wait_heads(0, 24, G, last_sems.at[1])
    tick = spread_queue(0, G, transpose_keys, range(3 * G, 4 * G), 2)
    p = {2: p_last(2, tick)}
    p[3] = probabilities(queries(B - 1, 3), lambda h: _bf16(r["k"][H + 3 * G + h]), True, tick)
    for i, (h0, n) in enumerate(LAST_HEADS[:-1]):
        wait_heads(1, h0, n, last_sems.at[2 + i])
        g = h0 // G
        a = a + outputs(p[g], H + g * G, g, range(h0 % G, h0 % G + n), idle)
    x = jnp.broadcast_to(r["x"][B - 1:B, :], (B, D)) + _row_sum(a)
    wait_heads(1, H - 1, 1, last_sems.at[1 + len(LAST_HEADS)])
    o = _row(_dot(p[3][0], _bf16(r["v"][2 * H - 1])) / p[3][1], G - 1)
    x = x + _dot(o.astype(bf16), _bf16(r["wo"][(H - 1) * 64:H * 64, :]))

    def fence():
        pl.semaphore_signal(fence_sem, 1)
        pl.semaphore_wait(fence_sem, 1)

    x = _mlp_one_row(x, r)
    fence()
    x = _attention_one_row(x, r)
    fence()
    x = _mlp_one_row(x, r)
    r["out"][...] = jnp.where(row_d == B - 1, x, r["x"][...]).astype(bf16)
    done = copy(r["out"], out_hbm, w_sems.at[0])
    done.start()
    done.wait()


def _call(A_x, A_k_cache, A_v_cache, A_wq, A_wo, B_w1, B_b1, B_w2, B_b2):
    out = pl.pallas_call(
        _kernel,
        in_specs=[pl.BlockSpec(memory_space=pl.ANY)] * 9,
        out_specs=pl.BlockSpec(memory_space=pl.ANY),
        out_shape=jax.ShapeDtypeStruct((B, D), bf16),
        scratch_shapes=[pltpu.VMEM(shape, dtype) for shape, dtype in SCRATCH.values()] + [
            pltpu.SemaphoreType.DMA((2, 8)),
            pltpu.SemaphoreType.DMA((7,)),
            pltpu.SemaphoreType.DMA((2 + len(LAST_HEADS),)),
            pltpu.SemaphoreType.REGULAR,
        ],
        compiler_params=pltpu.CompilerParams(
            vmem_limit_bytes=120 * 1024 * 1024,
            disable_bounds_checks=True,
            disable_semaphore_checks=True,
        ),
    )(
        A_x.reshape(B, D),
        A_k_cache.reshape(B * H, SK, DH),
        A_v_cache.reshape(B * H, SK, DH),
        A_wq.reshape(4, D // 4, H * DH),
        A_wo.reshape(4, H * DH // 4, D),
        B_w1.T.reshape(3, F // 3, D),
        B_b1,
        B_w2.reshape(3, F // 3, D),
        B_b2,
    )
    return out.reshape(B, 1, D)


@jax.jit
def pallas_interleave_layers__sliding_block_cached__mixer_channel_mlp__decode_kernel(
    A_x: jax.Array,
    A_k_cache: jax.Array,
    A_v_cache: jax.Array,
    A_wq: jax.Array,
    A_wo: jax.Array,
    B_x: jax.Array,
    B_w1: jax.Array,
    B_b1: jax.Array,
    B_w2: jax.Array,
    B_b2: jax.Array,
):
    del B_x
    return _call(A_x, A_k_cache, A_v_cache, A_wq, A_wo, B_w1, B_b1, B_w2, B_b2)
```

```python
import functools
import math

import jax
import jax.numpy as jnp
from jax import lax
import jax.experimental.pallas as pl
import jax.experimental.pallas.tpu as pltpu

f32, bf16, i32 = jnp.float32, jnp.bfloat16, jnp.int32

B, D, H, DH, SK, F = 8, 640, 32, 128, 4096, 1728
W = min(4096, max(256, SK // 4))
FP = 1792
G = 8
EPS = 1e-5
EXP2_SCALE = DH ** -0.5 * math.log2(math.e)
GELU_C = math.sqrt(2.0 / math.pi)

PAIRS_ATTN = 20
PAIRS_MLP = 40
PAIRS_REST = 256 - 8 * PAIRS_ATTN - PAIRS_MLP
LEAD = 128 - PAIRS_ATTN - PAIRS_MLP
LAST_HEADS = ((16, 4), (20, 4), (24, 5), (29, 2), (31, 1))

UP_MXU = 6
DOWN_MXU = 11
Q_MXU = (0, 1, 2)
O_MXU = (29, 30, 31)
PV_VPU = (0, 1, 2, 4, 6, 7, 10, 11, 12, 14)
SOFTMAX_GROUPS = (4, 4, 8, 8, 8)
PARTIAL_SUM = "33303233203331301201201201201201"
KT_PAD = 128

MLP_ORDER = """
    a0 a2 a1 t6 t10 a4 a3 t7 t8 c11 a5 t9 b1 b0 b2 a6 a7 a8 b3 a9 a10 c0 c1 d1 c2 b4 d2 c3 c4 d3 d4 b5 c16
    c5 c7 d5 c6 d6 d7 b6 c8 d8 c9 d9 c10 b7 d10 d11 c12 d12 b8 c13 d13 c14 d14 c15 d15 b9 d16 c17 d17 c18
    b10 d18 c19 d20 d19
"""
ATTENTION_ORDER = """
    q0 q1 q2 Q3 s0 Q4 q4 s1 Q5 s2 q3 s3 s4 q5 Q6 Q8 s5 Q7 Q9 q6 s6 q7 Q10 s7 q10 q8 Q11 q9 Q12 s9 s8 Q13 s10
    q11 s11 Q14 Q15 q12 s12 Q16 q16 q15 q13 Q18 Q17 q14 s14 s13 s15 Q19 s16 q17 s17 Q20 q18 Q21 q19 Q25 Q22
    q20 s19 Q24 s20 q21 Q23 q22 Q30 s22 s18 q23 Q26 Q27 q24 s23 Q28 q25 s24 s25 s21 q26 p0 q27 Q29 s26 s27
    q28 Q31 s28 w0_0 q29 q30 s30 x0_0 q31 p1 w1_0 s31 s29 w0_1 w0_2 w0_3 w2_0 x1_0 w1_1 w1_2 w1_3 p2 w2_1
    x0_1 x0_2 v3 x0_3 x2_0 x1_1 w2_2 x1_2 x1_3 w2_3 x2_1 v8 w4_0 w4_1 w4_2 v5 w4_3 v9 w6_0 w6_1 p3 w6_2 x2_2
    v13 x2_3 x4_0 x4_1 x4_2 x4_3 x6_0 v15 x6_1 x6_2 w6_3 w10_0 w10_1 v16 w10_2 w10_3 w11_0 w11_1 v17 w11_2
    x6_3 x10_0 w11_3 x10_1 x10_2 v18 x11_0 x11_1 x11_2 x11_3 c3 c5 v19 w12_0 w12_1 w12_2 w14_0 x14_0 v20
    w14_1 w12_3 w14_2 w14_3 x12_0 x12_1 x12_2 p4 x12_3 v21 c8 o3 x14_1 v22 x14_2 x14_3 c9 c13 v23 x10_3 c16
    c15 o5 w7_0 w7_1 w7_2 w7_3 x7_0 x7_1 x7_2 x7_3 v24 o8 o9 v25 c17 c19 o15 o13 c20 c21 c18 v27 c22 c23 o16
    o19 o17 v26 o18 c24 c27 v28 c25 c28 c26 o22 o20 o21 v30 v29 o23 o24 o25 v31 o26 o29 o27 o30 o28 o31
"""

SCRATCH = dict(
    k=((2 * H, W, DH), bf16),
    v=((2 * H, W, DH), bf16),
    v_last=((H, W // 2, DH), i32),
    kt_a=((H - G, DH // 2, W + KT_PAD), i32),
    kt_b=((G, DH // 2, W + KT_PAD), i32),
    wq_in=((4, D // 4, H * DH), bf16),
    wo_in=((4, H * DH // 4, D), bf16),
    w1_in=((3, F // 3, D), bf16),
    w2_in=((3, F // 3, D), bf16),
    wq=((D // 2, H * DH), i32),
    wo=((H * DH // 2, D), i32),
    w1=((D // 2, FP), i32),
    w2=((FP // 2, D), i32),
    wq_t_f32=((H * DH, D), f32),
    wo_f32=((H * DH, D), f32),
    w1_t_f32=((F - 128 * UP_MXU, D), f32),
    w1_sum=((B, FP), f32),
    wq_sum=((B, H * DH), f32),
    w2_half_f32=((F - 128 * DOWN_MXU, D), f32),
    b1_col=((FP - 128 * DOWN_MXU, 128), f32),
    x_in=((B, D), bf16),
    b1_in=((F,), bf16),
    b2_in=((D,), bf16),
    b1=((B, FP), f32),
    b2=((B, D), f32),
    x=((B, D), f32),
    out=((B, D), bf16),
    w1_sum_col=((FP - 128 * DOWN_MXU, 128), f32),
    q=((H * B + B, DH), f32),
    acc=((2, G, D), f32),
    vt_f32=((len(PV_VPU), DH, W), f32),
)


def _dot(a, b, transpose_b=False):
    dims = (((1,), (1 if transpose_b else 0,)), ((), ()))
    return lax.dot_general(a, b, dims, preferred_element_type=f32)


def _bf16(words):
    return pltpu.bitcast(words, bf16)


def _words(x):
    return pltpu.bitcast(x, i32)


def _tiles(x):
    return [x[:, k * 128:(k + 1) * 128] for k in range(x.shape[1] // 128)]


def _tile(ref, k):
    return ref[:, k * 128:(k + 1) * 128]


def _chain_sum(xs):
    return functools.reduce(lambda a, b: a + b, xs)


def _tree_sum(xs):
    while len(xs) > 1:
        xs = [_chain_sum(xs[i:i + 2]) for i in range(0, len(xs), 2)]
    return xs[0]


def _row_sum(x):
    return jnp.broadcast_to(jnp.sum(x, axis=0, keepdims=True), x.shape)


def _lane_sum(x):
    return jnp.broadcast_to(jnp.sum(x, axis=1, keepdims=True), x.shape)


def _row(x, j):
    return jnp.broadcast_to(x[j:j + 1, :], x.shape)


def _layernorm(x):
    c = x - jnp.mean(x, axis=-1, keepdims=True)
    return c * lax.rsqrt(jnp.mean(c * c, axis=-1, keepdims=True) + EPS)


def _gelu_twice(x):
    return x * jnp.tanh(x * (x * x * (GELU_C * 0.044715) + GELU_C)) + x


def _mean_var(x):
    xt = _tiles(x)
    mean = _lane_sum(_tree_sum(xt)) * (1.0 / D)
    return mean, _lane_sum(_tree_sum([(t - mean) * (t - mean) for t in xt])) * (1.0 / D)


def _run(steps, order):
    assert sorted(order.split()) == sorted(steps)
    for name in order.split():
        steps[name]()


def _mlp_one_row(x, r):
    mean, var = _mean_var(x)
    xt = _tiles(x)
    s1 = lax.rsqrt(var + EPS)
    scale = s1 * lax.rsqrt(var * s1 * s1 + EPS)
    xb = x.astype(bf16)
    hid, part, pre, z_m, z_v = {}, {}, {}, {}, {}

    def activate(j, t):
        hid[j] = 0.5 * _gelu_twice((t - mean * _tile(r["w1_sum"], j)) * scale + _tile(r["b1"], j))

    def up_rows(u):
        return _chain_sum([r["w1_t_f32"][u * 8:(u + 1) * 8, k * 128:(k + 1) * 128] * xt[k] for k in range(5)])

    def up_m(j):
        activate(j, _dot(xb, _bf16(_tile(r["w1"], j))))

    def up_v(j):
        part[j] = jnp.concatenate([up_rows((j - UP_MXU) * 16 + u) for u in range(16)], axis=0).T

    def up_v_finish(j):
        activate(j, _row_sum(_chain_sum([part[j][u * 8:(u + 1) * 8] for u in range(16)])))

    def down_m(j):
        for k, t in enumerate(_tiles(_dot(hid[j].astype(bf16), _bf16(r["w2"][j * 64:(j + 1) * 64, :])))):
            z_m[k] = t if k not in z_m else z_m[k] + t

    def up_col(us):
        for u in us:
            pre[u] = _lane_sum(up_rows((DOWN_MXU - UP_MXU) * 16 + u))

    def down_v(us):
        for u in us:
            rows = slice(u * 8, (u + 1) * 8)
            h = _gelu_twice((pre[u] - mean * r["w1_sum_col"][rows, :]) * scale + r["b1_col"][rows, :])
            for k in range(5):
                t = r["w2_half_f32"][rows, k * 128:(k + 1) * 128] * h
                z_v[k, u % 2] = t if (k, u % 2) not in z_v else z_v[k, u % 2] + t

    bind, steps = functools.partial, {}
    for j in range(DOWN_MXU):
        steps[f"a{j}"] = bind(up_m if j < UP_MXU else up_v_finish, j)
        steps[f"b{j}"] = bind(down_m, j)
        if j >= UP_MXU:
            steps[f"t{j}"] = bind(up_v, j)
    for i in range((F - DOWN_MXU * 128) // 16):
        steps[f"c{i}"] = bind(up_col, (2 * i, 2 * i + 1))
        steps[f"d{i + 1}"] = bind(down_v, (2 * i, 2 * i + 1))
    _run(steps, MLP_ORDER)
    base = _tiles(x + r["b2"][...])
    return jnp.concatenate([base[k] + _row_sum(z_v[k, 0] + z_v[k, 1]) + z_m[k] for k in range(5)], axis=1)


def _keys_t(r, h):
    return _bf16(r["kt_a"][h, :, :W] if h < H - G else r["kt_b"][h - (H - G), :, :W])


def _attention_one_row(x, r):
    row = lax.broadcasted_iota(i32, (8, 128), 0)
    mean, var = _mean_var(x)
    scale = lax.rsqrt(var + EPS) * EXP2_SCALE
    xb, xt = x.astype(bf16), _tiles(x)
    q, part, s, p, o, col, p_rows, z = {}, {}, {}, {}, {}, {}, {}, {}
    groups, place = [], {}
    for g, n in enumerate(SOFTMAX_GROUPS):
        groups.append(list(range(len(place), len(place) + n)))
        place.update({h: (g, j) for j, h in enumerate(groups[-1])})

    def diagonal(ts):
        out = ts[0]
        for k in range(1, len(ts)):
            out = jnp.where(row == k, ts[k], out)
        return out

    def add(key, t):
        z[key] = t if key not in z else z[key] + t

    def query_m(h):
        q[h] = _dot(xb, _bf16(_tile(r["wq"], h))) - mean * _tile(r["wq_sum"], h)

    def query_v(h):
        def rows(u):
            n = h * DH + u * 8
            return _chain_sum([r["wq_t_f32"][n:n + 8, k * 128:(k + 1) * 128] * xt[k] for k in range(5)])
        part[h] = jnp.concatenate([rows(u) for u in range(16)], axis=0).T

    def query_v_finish(h):
        t = _row_sum(_chain_sum([part[h][u * 8:(u + 1) * 8] for u in range(16)]))
        q[h] = t - mean * _tile(r["wq_sum"], h)

    def scores(h):
        s[h] = diagonal(_tiles(_dot(q[h].astype(bf16), _keys_t(r, h))))

    def softmax(hs):
        m = diagonal([jnp.broadcast_to(jnp.max(s[h], axis=0, keepdims=True), (8, 128)) for h in hs])
        m = jnp.broadcast_to(jnp.max(m, axis=1, keepdims=True), (8, 128))
        e = [jnp.exp2((s[h] - m[j:j + 1, :]) * scale) for j, h in enumerate(hs)]
        inv = 1.0 / _lane_sum(diagonal([_row_sum(t) for t in e]))
        for j, h in enumerate(hs):
            p[h] = (e[j], inv)

    def values_m(h):
        j = place[h][1]
        pb = p[h][0].astype(bf16)
        t = diagonal([_dot(pb, _bf16(r["v_last"][h, k * 64:(k + 1) * 64, :])) for k in range(8)])
        t = t * p[h][1][j:j + 1, :]
        o[h] = t if h in O_MXU else _row_sum(t)

    def values_v(h, i):
        if i == 0:
            j = place[h][1]
            e = p[h][0] * p[h][1][j:j + 1, :]
            p_rows[h] = [_row(e, k) for k in range(8)]
        for u in range(4 * i, 4 * i + 4):
            t = [r["vt_f32"][PV_VPU.index(h), u * 8:(u + 1) * 8, k * 128:(k + 1) * 128] * p_rows[h][k]
                 for k in range(8)]
            col[h, u] = _lane_sum(_chain_sum(t[:4]) + _chain_sum(t[4:]))

    def to_columns(h):
        t = jnp.concatenate([o[h]] * 16, axis=0).T
        for u in range(16):
            col[h, u] = t[u * 8:(u + 1) * 8]

    def output_m(h):
        for k, t in enumerate(_tiles(_dot(o[h].astype(bf16), _bf16(r["wo"][h * 64:(h + 1) * 64, :])))):
            add((k, "M"), t)

    def output_v(h, us):
        for u in us:
            n = h * DH + u * 8
            for k in range(5):
                add((k, PARTIAL_SUM[h]), r["wo_f32"][n:n + 8, k * 128:(k + 1) * 128] * col[h, u])

    bind, steps = functools.partial, {}
    for h in range(H):
        steps[f"q{h}"] = bind(query_m if h in Q_MXU else query_v_finish, h)
        if h not in Q_MXU:
            steps[f"Q{h}"] = bind(query_v, h)
        steps[f"s{h}"] = bind(scores, h)
        if h in PV_VPU:
            for i in range(4):
                steps[f"w{h}_{i}"] = bind(values_v, h, i)
                steps[f"x{h}_{i}"] = bind(output_v, h, range(4 * i, 4 * i + 4))
            continue
        steps[f"v{h}"] = bind(values_m, h)
        if h in O_MXU:
            steps[f"o{h}"] = bind(output_m, h)
        else:
            steps[f"c{h}"] = bind(to_columns, h)
            steps[f"o{h}"] = bind(output_v, h, range(16))
    for g, hs in enumerate(groups):
        steps[f"p{g}"] = bind(softmax, hs)
    _run(steps, ATTENTION_ORDER)
    return x + jnp.concatenate([_row_sum(_tree_sum([z[k, e] for e in "0123M" if (k, e) in z])) for k in range(5)], axis=1)


def _kernel(x_hbm, k_hbm, v_hbm, wq_hbm, wo_hbm, w1_hbm, b1_hbm, w2_hbm, b2_hbm, out_hbm, *scratch):
    r = dict(zip(SCRATCH, scratch))
    kv_sems, w_sems, last_sems, fence_sem = scratch[len(SCRATCH):]
    copy = pltpu.make_async_copy
    kv_src = (k_hbm, v_hbm)
    kv_dst = (r["k"], r["v"])
    row = lax.broadcasted_iota(i32, (G, DH), 0)
    row_d = lax.broadcasted_iota(i32, (B, D), 0)

    def start_pair(m):
        group, h, key = m >> 6, (m & 3) * 2, ((m >> 2) & 15) * 64
        if not isinstance(key, int):
            key = pl.multiple_of(key, 64)
        for t in range(2):
            copy(kv_src[t].at[pl.ds(group * G + h, 2), pl.ds(SK - W + key, 64)],
                 kv_dst[t].at[pl.ds((group & 7) * G + h, 2), pl.ds(key, 64)],
                 kv_sems.at[t, group & 7]).start(priority=t)

    def start_pairs(m, n):
        def body(i, _):
            for c in range(4):
                start_pair(m + i * 4 + c)
        lax.fori_loop(0, n // 4, body, None)

    def spread_pairs(m, n, points):
        calls = [0]
        def tick():
            for c in range(n * calls[0] // points, n * (calls[0] + 1) // points):
                start_pair(m + c)
            calls[0] += 1
        return tick

    def wait_group(t, group):
        ref = kv_dst[t].at[pl.ds((group & 7) * G, G)]
        copy(ref, ref, kv_sems.at[t, group & 7]).wait()

    def idle():
        pass

    def queries(b, g):
        return r["q"][pl.ds(g * (G * B) + b, G, stride=B), :].astype(bf16)

    def probabilities(q, keys, transpose, tick):
        s = [None] * (W // 128)
        for h in range(G):
            for j, t in enumerate(_tiles(_dot(q, keys(h), transpose))):
                s[j] = t if h == 0 else jnp.where(row == h, t, s[j])
            tick()
        s = jnp.concatenate(s, axis=1)
        p = jnp.exp2((s - jnp.max(s, axis=1, keepdims=True)) * EXP2_SCALE)
        return p.astype(bf16), jnp.sum(p, axis=1, keepdims=True)

    def outputs(p, values, g, heads, tick):
        o = None
        for h in heads:
            t = _dot(p[0], values(h))
            o = t if o is None else jnp.where(row == h, t, o)
            tick()
        o = (o / p[1]).astype(bf16)
        out = None if len(heads) == G else jnp.zeros((G, D), f32)
        for h in heads:
            w = (g * G + h) * 64
            if not isinstance(w, int):
                w = pl.multiple_of(w, 64)
            t = _dot(o, _bf16(r["wo"][pl.ds(w, 64), :]))
            out = t if out is None else jnp.where(row_d == h, t, out)
            tick()
        return out

    def mlp(x, tick):
        y = _layernorm(_layernorm(x)).astype(bf16)
        edges = [(c, min(c + 512, FP)) for c in range(0, FP, 512)]
        hid = []
        for lo, hi in edges:
            hid.append((0.5 * _gelu_twice(_dot(y, _bf16(r["w1"][:, lo:hi])) + r["b1"][:, lo:hi])).astype(bf16))
            tick()
        out = x + r["b2"][...]
        for h, (lo, hi) in zip(hid, edges):
            out = out + _dot(h, _bf16(r["w2"][lo // 2:hi // 2, :]))
            tick()
        return out

    def project_queries(tick):
        y = _layernorm(r["x"][...]).astype(bf16)
        for c in range(8):
            for j, t in enumerate(_tiles(_dot(y, _bf16(r["wq"][:, c * 512:(c + 1) * 512])))):
                r["q"][(c * 4 + j) * B:(c * 4 + j + 1) * B, :] = t
            tick()

    def load_wq_wo(i, _):
        rows = pl.ds(pl.multiple_of((i >> 3) * 8, 8), 8)
        cols = pl.ds(pl.multiple_of((i & 7) * 512, 512), 512)
        copy(wq_hbm.at[:, rows, cols], r["wq_in"].at[:, rows, cols], w_sems.at[3]).start(priority=0)

        @pl.when(i < H * DH // 4 // 8)
        def _():
            rows = pl.ds(pl.multiple_of(i * 8, 8), 8)
            copy(wo_hbm.at[:, rows], r["wo_in"].at[:, rows], w_sems.at[4]).start(priority=1)

    def load_w1_w2(i, _):
        rows = pl.ds(pl.multiple_of(i * 8, 8), 8)
        copy(w1_hbm.at[:, rows], r["w1_in"].at[:, rows], w_sems.at[5]).start(priority=0)
        copy(w2_hbm.at[:, rows], r["w2_in"].at[:, rows], w_sems.at[6]).start(priority=1)

    small = [copy(x_hbm, r["x_in"], w_sems.at[0]), copy(b1_hbm, r["b1_in"], w_sems.at[1]),
             copy(b2_hbm, r["b2_in"], w_sems.at[2])]
    lax.fori_loop(0, D // 4, load_wq_wo, None)
    for c in small:
        c.start()
    lax.fori_loop(0, F // 3 // 8, load_w1_w2, None)

    def wait_weight(name, i):
        copy(r[name], r[name], w_sems.at[i]).wait()

    def columns(ref, bias):
        for j in range(DOWN_MXU, FP // 128):
            t = jnp.broadcast_to(bias[0:1, j * 128:(j + 1) * 128], (128, 128)).T
            ref[(j - DOWN_MXU) * 128:(j - DOWN_MXU + 1) * 128, :] = t

    for c in small:
        c.wait()
    r["acc"][...] = jnp.zeros((2, G, D), f32)
    r["q"][H * B:, :] = jnp.zeros((B, DH), f32)
    r["x"][...] = r["x_in"][...].astype(f32)
    b1 = jnp.concatenate([r["b1_in"][...].astype(f32).reshape(1, F), jnp.zeros((1, FP - F), f32)], axis=1)
    r["b1"][...] = jnp.broadcast_to(b1, (B, FP))
    columns(r["b1_col"], b1)
    r["b2"][...] = jnp.broadcast_to(r["b2_in"][...].astype(f32).reshape(1, D), (B, D))

    def pack_wq(i, _):
        for a in range(4):
            rows = pl.ds(pl.multiple_of(a * (D // 8) + i * 8, 8), 8)
            r["wq"][rows, :] = _words(r["wq_in"][a, pl.ds(pl.multiple_of(i * 16, 16), 16), :])
            if a % 2:
                start_pair(i * 2 + a // 2)

    def transpose_wq(i, _):
        for e in range(2):
            head = pl.ds(pl.multiple_of((2 * i + e) * DH, DH), DH)
            r["wq_t_f32"][head, :] = _bf16(r["wq"][:, head]).T.astype(f32)
            for c in range(2 + 2 * e):
                start_pair(36 + i * 6 + 2 * e + c)

    def pack_wo(i, _):
        for a in range(4):
            w = r["wo_in"][a, pl.ds(pl.multiple_of(i * DH, DH), DH), :]
            r["wo"][pl.ds(pl.multiple_of((a * 8 + i) * 64, 64), 64), :] = _words(w)
            r["wo_f32"][pl.ds(pl.multiple_of((a * 8 + i) * DH, DH), DH), :] = w.astype(f32)
            start_pair(132 + i * 4 + a)

    wait_weight("wq_in", 3)
    lax.fori_loop(0, 10, pack_wq, None)
    project_queries(spread_pairs(20, 16, 8))
    lax.fori_loop(0, H // 2, transpose_wq, None)
    wait_weight("wo_in", 4)
    lax.fori_loop(0, 8, pack_wo, None)

    def mlp_rows(name, n):
        return r[name][n // (F // 3), n % (F // 3):n % (F // 3) + 64, :]

    loop_start = LEAD + 256 - PAIRS_REST - 3 * PAIRS_ATTN
    tick = spread_pairs(164, loop_start - 164, 9 + 14 + 8)
    wait_weight("w2_in", 6)
    for n in range(0, F, 64):
        w = mlp_rows("w2_in", n)
        r["w2"][n // 2:n // 2 + 32, :] = _words(w)
        if n >= 128 * DOWN_MXU:
            r["w2_half_f32"][n - 128 * DOWN_MXU:n - 128 * DOWN_MXU + 64, :] = 0.5 * w.astype(f32)
        if n % 192 == 0:
            tick()
    r["w2"][F // 2:, :] = jnp.zeros(((FP - F) // 2, D), i32)
    wait_weight("w1_in", 5)
    for c in range(FP // 128):
        halves = []
        for n in (c * 128, c * 128 + 64):
            halves.append(mlp_rows("w1_in", n) if n < F else jnp.zeros((64, D), bf16))
            if 128 * UP_MXU <= n < F:
                r["w1_t_f32"][n - 128 * UP_MXU:n - 128 * UP_MXU + 64, :] = halves[-1].astype(f32)
        r["w1"][:, c * 128:(c + 1) * 128] = _words(jnp.concatenate(halves, axis=0).T)
        tick()
    ones = jnp.ones((B, D), bf16)
    w1_sum = _dot(ones, _bf16(r["w1"][...]))
    r["w1_sum"][...] = w1_sum
    columns(r["w1_sum_col"], w1_sum)
    for c in range(8):
        r["wq_sum"][:, c * 512:(c + 1) * 512] = _dot(ones, _bf16(r["wq"][:, c * 512:(c + 1) * 512]))
        tick()

    def step(j, total):
        s, i = j >> 3, j & 7
        first = i >= 4
        b, g = jnp.where(first, s, s - 1), i & 3
        m = LEAD + 256 * (s + 1) + PAIRS_ATTN * (i - 7)

        @pl.when(i == 7)
        def _():
            start_pairs(m - PAIRS_REST, PAIRS_REST)

        @pl.when(first)
        def _():
            wait_group(0, b * 4 + g)
            wait_group(1, b * 4 + g)

        tick = spread_pairs(jnp.where(i == 7, m, m - PAIRS_REST), PAIRS_ATTN, 3 * G)
        slot = (b & 1) * H + g * G
        p = probabilities(queries(b, g), lambda h: r["k"][slot + h], True, tick)
        r["acc"][jnp.where(first, 0, 1)] += outputs(p, lambda h: r["v"][slot + h], g, range(G), tick)

        @pl.when(i == 7)
        def _():
            tick = spread_pairs(m + PAIRS_ATTN, PAIRS_MLP, 16)
            a1 = jnp.sum(r["acc"][0], axis=0, keepdims=True)
            a2 = jnp.sum(r["acc"][1], axis=0, keepdims=True)
            x = r["x"][...]
            r["acc"][...] = jnp.zeros((2, G, D), f32)
            y = mlp(x + jnp.where(row_d == s, a1, a2), tick)
            r["x"][...] = jnp.where((row_d == s) | (row_d == s - 1), y, x)
            project_queries(tick)

        return total + j

    zero = lax.fori_loop(4, 8 * (B - 1), step, 0) - sum(range(4, 8 * (B - 1)))

    queue = []

    def plan(t, h, n, key, keys, sem, thread):
        c = copy(kv_src[t].at[pl.ds((B - 1) * H + h, n), pl.ds(SK - W + key, keys)],
                 kv_dst[t].at[pl.ds(H + h, n), pl.ds(key, keys)], sem)
        queue.append(functools.partial(c.start, priority=thread))

    def values_sem(h):
        return last_sems.at[2 + [h0 <= h < h0 + n for h0, n in LAST_HEADS].index(True)]

    def wait_heads(t, h, n, sem):
        ref = kv_dst[t].at[pl.ds(H + h, n)]
        copy(ref, ref, sem).wait()

    for e in range(2):
        for i in range(32):
            for thread in range(2):
                plan(0, 16 + 8 * e + 4 * thread + 2 * (i % 2), 2, 64 * (i // 2), 64, last_sems.at[e], thread)
    for i in range(32):
        for thread in range(2):
            plan(1, 16 + 4 * thread + 2 * (i % 2), 2, 64 * (i // 2), 64, values_sem(16 + 4 * thread), thread)
    for i in range(32):
        plan(1, 24 + 2 * (i % 2), 2, 64 * (i // 2), 64, values_sem(24), 0)
        plan(1, 28 + i // 8, 1, 128 * (i % 8), 128, values_sem(28 + i // 8), 1)

    def transpose_keys(h):
        ref = r["kt_a"] if h < H - G else r["kt_b"]
        ref[zero + h % (H - G), :, :W] = _words(r["k"][H + h].T)

    def transpose_values(h):
        r["vt_f32"][zero + PV_VPU.index(h)] = r["v"][H + h].T.astype(f32)

    def spread_queue(pairs, points, side_job=None, heads=(), every=1):
        calls, heads = [0], list(heads)
        def tick():
            for _ in range(2 * (pairs * (calls[0] + 1) // points - pairs * calls[0] // points)):
                queue.pop(0)()
            if heads and calls[0] % every == 0:
                side_job(heads.pop(0))
            calls[0] += 1
        return tick

    def p_prev(g, tick):
        return probabilities(queries(B - 2, g), lambda h: r["k"][g * G + h], True, tick)

    def o_prev(g, p, tick):
        return outputs(p, lambda h: r["v"][g * G + h], g, range(G), tick)

    p0 = p_prev(0, spread_queue(10, G))
    wait_group(0, 4 * (B - 1))
    tick = spread_queue(30, 4 * G, transpose_keys, range(G), 4)
    p1 = p_prev(1, tick)
    a = o_prev(0, p0, tick)
    p2 = p_prev(2, tick)
    wait_group(0, 4 * (B - 1) + 1)
    tick = spread_queue(34, 7 * G, transpose_keys, range(G, 2 * G), 7)
    a = a + o_prev(1, p1, tick)
    p3 = p_prev(3, tick)
    a = a + o_prev(2, p2, tick) + o_prev(3, p3, tick)

    def p_last(g, tick):
        return probabilities(queries(B - 1, g), lambda h: _keys_t(r, g * G + h), False, tick)

    def keep_values(h):
        v = r["v"][H + h]
        if h not in PV_VPU:
            r["v_last"][zero + h] = _words(v)
        return v

    def o_last(g, p, heads, tick):
        return outputs(p, lambda h: keep_values(g * G + h), g, heads, tick)

    wait_group(1, 4 * (B - 1))
    wait_group(1, 4 * (B - 1) + 1)
    tick = spread_queue(22, 2 * G, transpose_values, PV_VPU)
    p0, p1 = p_last(0, tick), p_last(1, tick)
    x = r["x"][...]
    r["x"][...] = jnp.where(row_d == B - 2, mlp(x + jnp.sum(a, axis=0, keepdims=True), idle), x)
    wait_heads(0, 16, G, last_sems.at[0])
    tick = spread_queue(18, 4 * G, transpose_keys, range(2 * G, 3 * G), 4)
    a = o_last(0, p0, range(G), tick) + o_last(1, p1, range(G), tick)
    while queue:
        queue.pop(0)()
    wait_heads(0, 24, G, last_sems.at[1])
    tick = spread_queue(0, G, transpose_keys, range(3 * G, 4 * G), 2)
    p = {2: p_last(2, tick)}
    p[3] = probabilities(queries(B - 1, 3), lambda h: r["k"][H + 3 * G + h], True, tick)
    for i, (h0, n) in enumerate(LAST_HEADS[:-1]):
        wait_heads(1, h0, n, last_sems.at[2 + i])
        a = a + o_last(h0 // G, p[h0 // G], range(h0 % G, h0 % G + n), idle)
    x = jnp.broadcast_to(r["x"][B - 1:B, :], (B, D)) + _row_sum(a)
    wait_heads(1, H - 1, 1, last_sems.at[1 + len(LAST_HEADS)])
    o = _row(_dot(p[3][0], keep_values(H - 1)) / p[3][1], G - 1)
    x = x + _dot(o.astype(bf16), _bf16(r["wo"][(H - 1) * 64:H * 64, :]))

    def fence():
        pl.semaphore_signal(fence_sem, 1)
        pl.semaphore_wait(fence_sem, 1)

    x = _mlp_one_row(x, r)
    fence()
    x = _attention_one_row(x, r)
    fence()
    x = _mlp_one_row(x, r)
    r["out"][...] = jnp.where(row_d == B - 1, x, r["x"][...]).astype(bf16)
    done = copy(r["out"], out_hbm, w_sems.at[0])
    done.start()
    done.wait()


def _call(A_x, A_k_cache, A_v_cache, A_wq, A_wo, B_w1, B_b1, B_w2, B_b2):
    out = pl.pallas_call(
        _kernel,
        in_specs=[pl.BlockSpec(memory_space=pl.ANY)] * 9,
        out_specs=pl.BlockSpec(memory_space=pl.ANY),
        out_shape=jax.ShapeDtypeStruct((B, D), bf16),
        scratch_shapes=[pltpu.VMEM(shape, dtype) for shape, dtype in SCRATCH.values()] + [
            pltpu.SemaphoreType.DMA((2, 8)),
            pltpu.SemaphoreType.DMA((7,)),
            pltpu.SemaphoreType.DMA((2 + len(LAST_HEADS),)),
            pltpu.SemaphoreType.REGULAR,
        ],
        compiler_params=pltpu.CompilerParams(
            vmem_limit_bytes=120 * 1024 * 1024,
            disable_bounds_checks=True,
            disable_semaphore_checks=True,
        ),
    )(
        A_x.reshape(B, D),
        A_k_cache.reshape(B * H, SK, DH),
        A_v_cache.reshape(B * H, SK, DH),
        A_wq.reshape(4, D // 4, H * DH),
        A_wo.reshape(4, H * DH // 4, D),
        B_w1.T.reshape(3, F // 3, D),
        B_b1,
        B_w2.reshape(3, F // 3, D),
        B_b2,
    )
    return out.reshape(B, 1, D)


@jax.jit
def pallas_interleave_layers__sliding_block_cached__mixer_channel_mlp__decode_kernel(
    A_x: jax.Array,
    A_k_cache: jax.Array,
    A_v_cache: jax.Array,
    A_wq: jax.Array,
    A_wo: jax.Array,
    B_x: jax.Array,
    B_w1: jax.Array,
    B_b1: jax.Array,
    B_w2: jax.Array,
    B_b2: jax.Array,
):
    del B_x
    return _call(A_x, A_k_cache, A_v_cache, A_wq, A_wo, B_w1, B_b1, B_w2, B_b2)
```
